```python
import os as _os
_os.environ.setdefault("JAX_PLATFORMS", "cpu")
import jax
import jax.numpy as jnp

def _softmax(x, axis=-1):
    return jax.nn.softmax(x, axis=axis)
def _gelu(x):
    return jax.nn.gelu(x, approximate=True)
def _silu(x):
    return jax.nn.silu(x)
def _sigmoid(x):
    return jax.nn.sigmoid(x)
def _layernorm(x, axis=-1, eps=1e-5):
    m = jnp.mean(x, axis=axis, keepdims=True)
    v = jnp.var(x, axis=axis, keepdims=True)
    return (x - m) / jnp.sqrt(v + eps)
def _scatter_add(tgt, idx, src, axis=0):
    return tgt.at[idx].add(src)
def _segment_sum(src, seg, n):
    return jax.ops.segment_sum(src, seg, n)
class _Rng:
    def __init__(self, key):
        self._k = key
    def _next(self):
        self._k, sub = jax.random.split(self._k)
        return sub
    def normal(self, shape):
        return jax.random.normal(self._next(), shape, dtype=jnp.bfloat16)
    def randint(self, lo, hi, shape):
        return jax.random.randint(self._next(), shape, lo, hi, dtype=jnp.int32)
    def uniform(self, shape, lo=0.0, hi=1.0):
        return jax.random.uniform(self._next(), shape, jnp.bfloat16, lo, hi)
    def permutation(self, n):
        return jax.random.permutation(self._next(), n)


kernel_name = 'standalone__channel_attn_cbam__vision'

def setup_inputs():
    _rng = _Rng(jax.random.key(int.from_bytes(__import__("os").urandom(4), "little")))
    _w = (lambda a: (lambda t: t.astype(jnp.bfloat16) if jnp.issubdtype(t.dtype, jnp.floating) else t)(jnp.asarray(a)))
    H = W = 224
    C = 192
    r = max(C // 4, 1)
    return {
        "x": _w((lambda *s: _rng.normal(s) * 0.2)(1, H, W, C) + (lambda *s: _rng.normal(s) * 0.2)(1, 1, 1, C) * 2.0),
        "w1": _w((lambda *s: _rng.normal(s) * 0.2)(C, r)),
        "w2": _w((lambda *s: _rng.normal(s) * 0.2)(r, C)),
    }

def reference(x, w1, w2):
    B, H, W, C = x.shape
    xf = x.reshape(B, H * W, C)
    gap = jnp.mean(xf, 1)
    gmp = jnp.amax(xf, 1)
    h_a = gap @ w1
    h_a = h_a * (lambda x, dt: x.astype(dt))(h_a > 0, h_a.dtype)
    h_m = gmp @ w1
    h_m = h_m * (lambda x, dt: x.astype(dt))(h_m > 0, h_m.dtype)
    scale = _sigmoid(h_a @ w2 + h_m @ w2)
    return x * scale[:, None, None, :]
```

```python
import jax
import jax.numpy as jnp
from jax import lax
import jax.experimental.pallas as pl
import jax.experimental.pallas.tpu as pltpu

F32, BF16 = jnp.float32, jnp.bfloat16

CB = 16
HG = 32
ROWS = 48
HEAD = 16
UNROLL = 8
SLABS = (8, 2, 1)
LAST = ((0, 5, 0, 32), (5, 1, 0, 32), (6, 1, 0, 24), (6, 1, 24, 8))


def _rnd(a):
    return a.astype(BF16).astype(F32)


@jax.jit
def pallas_standalone__channel_attn_cbam__vision_kernel(
    x: jax.Array,
    w1: jax.Array,
    w2: jax.Array,
):
    B, H, W, C = x.shape
    R = w1.shape[1]
    S = H // HG
    P = C // ROWS
    assert B == 1 and S * HG == H and P * ROWS == C and R <= 64 and 128 < W <= 256

    reads = []
    c0 = 0
    for b in SLABS:
        reads.append((0, S, 0, HG, c0, b * CB))
        c0 += b * CB
    assert c0 == C - CB and sum(t[1] * t[3] for t in LAST) == H
    reads += [(*t, c0, CB) for t in LAST]

    def kernel(x_hbm, w1_hbm, w2_hbm, o_hbm, xbuf, w1b, w2b, w1d, w2d, gate_ref,
               rsem, wsem, psem):
        def rd(i):
            s0, sn, h0, hn, c0, cn = reads[i]
            idx = (pl.ds(s0, sn), pl.ds(h0, hn), pl.ds(c0, cn))
            return pltpu.make_async_copy(x_hbm.at[idx], xbuf.at[idx], rsem.at[i])

        def wr(hh, c0, cn):
            idx = (slice(None), hh, pl.ds(c0, cn))
            return pltpu.make_async_copy(xbuf.at[idx], o_hbm.at[idx], wsem)

        cw1 = pltpu.make_async_copy(w1_hbm, w1b, psem.at[0])
        cw2 = pltpu.make_async_copy(w2_hbm, w2b, psem.at[1])
        for i in range(len(reads)):
            rd(i).start(priority=1)
        cw1.start()
        cw2.start()
        cw1.wait()
        cw2.wait()

        def spread(wb):
            wf = wb[...].astype(F32)
            z = jnp.zeros((64 - R, C), F32)
            return jnp.concatenate([wf, z, wf, z], axis=0).T

        w1d[...] = spread(w1b)
        w2d[...] = spread(w2b)

        def pool(c0, s0, sn, h0, hn, s, m):
            def step(si, h, carry):
                s, m = carry
                v = xbuf[si, h, pl.ds(c0, CB), :].astype(F32)
                return s + v, jnp.maximum(m, v)

            if sn * hn <= 2 * UNROLL or hn % UNROLL:
                for si in range(s0, s0 + sn):
                    for h in range(h0, h0 + hn):
                        s, m = step(si, h, (s, m))
                return s, m
            nu = hn // UNROLL

            def body(t, carry):
                si = s0 + lax.div(t, nu)
                hb = h0 + lax.rem(t, nu) * UNROLL
                for u in range(UNROLL):
                    carry = step(si, hb + u, carry)
                return carry

            return lax.fori_loop(0, sn * nu, body, (s, m))

        def init():
            return jnp.zeros((CB, W), F32), jnp.full((CB, W), -jnp.inf, F32)

        lane = lax.broadcasted_iota(jnp.int32, (CB, 128), 1)

        def layer1(c0, s, m):
            gap = _rnd(jnp.sum(s, axis=1, keepdims=True) * (1.0 / (H * W)))
            gmp = jnp.max(m, axis=1, keepdims=True)
            return jnp.where(lane < 64, gap, gmp) * w1d[pl.ds(c0, CB), :]

        hacc = jnp.zeros((CB, 128), F32)
        for i, b in enumerate(SLABS):
            rd(i).wait()

            def slab_body(cb, hacc, base=reads[i][4]):
                c0 = pl.multiple_of(base + cb * CB, CB)
                s, m = pool(c0, 0, S, 0, HG, *init())
                return hacc + layer1(c0, s, m)

            hacc = lax.fori_loop(0, b, slab_body, hacc)
        s, m = init()
        for i in range(len(SLABS), len(reads)):
            rd(i).wait()
            s, m = pool(C - CB, *reads[i][:4], s, m)
        hacc = hacc + layer1(C - CB, s, m)
        h = _rnd(jnp.sum(hacc, axis=0, keepdims=True))
        h = h * (h > 0).astype(F32)

        def gate(c0, cn):
            z = _rnd(jnp.sum(w2d[pl.ds(c0, cn), :] * h, axis=1, keepdims=True))
            return jnp.broadcast_to(_rnd(jax.nn.sigmoid(z)), (cn, 128))

        def apply(hh, c0, g):
            g = jnp.concatenate([g, g[:, :W - 128]], axis=1)
            for si in range(S):
                v = xbuf[si, hh, pl.ds(c0, CB), :].astype(F32)
                xbuf[si, hh, pl.ds(c0, CB), :] = (v * g).astype(xbuf.dtype)

        head = [(0, HEAD), (HEAD, ROWS)]
        head += [(p * ROWS, (p + 1) * ROWS) for p in range(1, P)]
        for a, b in head:
            g = gate(a, b - a)
            gate_ref[pl.ds(a, b - a), :] = g
            for r in range(0, b - a, CB):
                apply(0, a + r, g[r:r + CB])
            wr(0, a, b - a).start()

        def row_body(hh, carry):
            for p in range(P):
                for r in range(p * ROWS, (p + 1) * ROWS, CB):
                    apply(hh, r, gate_ref[pl.ds(r, CB), :])
                wr(hh, p * ROWS, ROWS).start()
            return carry

        lax.fori_loop(1, HG, row_body, 0)
        pltpu.make_async_copy(xbuf, o_hbm, wsem).wait()

    xt = jnp.transpose(x, (0, 1, 3, 2)).reshape(S, HG, C, W)
    out = pl.pallas_call(
        kernel,
        out_shape=jax.ShapeDtypeStruct((S, HG, C, W), x.dtype),
        in_specs=[pl.BlockSpec(memory_space=pltpu.HBM)] * 3,
        out_specs=pl.BlockSpec(memory_space=pltpu.HBM),
        scratch_shapes=[
            pltpu.VMEM((S, HG, C, W), x.dtype),
            pltpu.VMEM((R, C), w1.dtype),
            pltpu.VMEM((R, C), w2.dtype),
            pltpu.VMEM((C, 128), F32),
            pltpu.VMEM((C, 128), F32),
            pltpu.VMEM((C, 128), F32),
            pltpu.SemaphoreType.DMA((len(reads),)),
            pltpu.SemaphoreType.DMA(()),
            pltpu.SemaphoreType.DMA((2,)),
        ],
        compiler_params=pltpu.CompilerParams(vmem_limit_bytes=64 * 1024 * 1024),
    )(xt, w1.T, w2)
    return jnp.transpose(out.reshape(B, H, C, W), (0, 1, 3, 2))
```

```python
import jax
import jax.numpy as jnp
from jax import lax
import jax.experimental.pallas as pl
import jax.experimental.pallas.tpu as pltpu

F32, BF16 = jnp.float32, jnp.bfloat16

CB = 16
HG = 32
SLABS = (8, 3)
LAST = (5, 1, 1)
OUT_C = 48


def _rnd(a):
    return a.astype(BF16).astype(F32)


@jax.jit
def pallas_standalone__channel_attn_cbam__vision_kernel(
    x: jax.Array,
    w1: jax.Array,
    w2: jax.Array,
):
    B, H, W, C = x.shape
    R = w1.shape[1]
    S = H // HG
    assert B == 1 and S * HG == H and C % OUT_C == 0 and R <= 64 and 128 < W <= 256

    reads = []
    c0 = 0
    for b in SLABS:
        reads.append((0, S, c0, b * CB))
        c0 += b * CB
    s0 = 0
    for n in LAST:
        reads.append((s0, n, c0, CB))
        s0 += n
    assert c0 == C - CB and s0 == S

    def kernel(x_hbm, w1_hbm, w2_hbm, o_hbm, xbuf, w1b, w2b, w1d, w2d, gate_ref,
               rsem, wsem, psem):
        def rd(i):
            s0, sn, c0, cn = reads[i]
            idx = (pl.ds(s0, sn), slice(None), pl.ds(c0, cn))
            return pltpu.make_async_copy(x_hbm.at[idx], xbuf.at[idx], rsem.at[i])

        def wr(hh, c0, cn):
            idx = (slice(None), hh, pl.ds(c0, cn))
            return pltpu.make_async_copy(xbuf.at[idx], o_hbm.at[idx], wsem)

        cw1 = pltpu.make_async_copy(w1_hbm, w1b, psem.at[0])
        cw2 = pltpu.make_async_copy(w2_hbm, w2b, psem.at[1])
        for i in range(len(reads)):
            rd(i).start(priority=1)
        cw1.start()
        cw2.start()
        cw1.wait()
        cw2.wait()

        def spread(wb):
            wf = wb[...].astype(F32)
            z = jnp.zeros((64 - R, C), F32)
            return jnp.concatenate([wf, z, wf, z], axis=0).T

        w1d[...] = spread(w1b)
        w2d[...] = spread(w2b)

        def pool(c0, s0, sn, acc):
            def group(si, acc):
                s, m = acc
                for hh in range(HG):
                    v = xbuf[si, hh, pl.ds(c0, CB), :].astype(F32)
                    s, m = s + v, jnp.maximum(m, v)
                return s, m

            if sn == 1:
                return group(s0, acc)
            return lax.fori_loop(s0, s0 + sn, group, acc)

        def init():
            return jnp.zeros((CB, W), F32), jnp.full((CB, W), -jnp.inf, F32)

        lane = lax.broadcasted_iota(jnp.int32, (CB, 128), 1)

        def layer1(c0, acc):
            s, m = acc
            gap = _rnd(jnp.sum(s, axis=1, keepdims=True) * (1.0 / (H * W)))
            gmp = jnp.max(m, axis=1, keepdims=True)
            return jnp.where(lane < 64, gap, gmp) * w1d[pl.ds(c0, CB), :]

        hacc = jnp.zeros((CB, 128), F32)
        for i, b in enumerate(SLABS):
            rd(i).wait()

            def block(cb, hacc, base=reads[i][2]):
                c0 = pl.multiple_of(base + cb * CB, CB)
                return hacc + layer1(c0, pool(c0, 0, S, init()))

            hacc = lax.fori_loop(0, b, block, hacc)
        acc = init()
        for i in range(len(SLABS), len(reads)):
            rd(i).wait()
            acc = pool(C - CB, reads[i][0], reads[i][1], acc)
        hacc = hacc + layer1(C - CB, acc)
        h = _rnd(jnp.sum(hacc, axis=0, keepdims=True))
        h = h * (h > 0).astype(F32)
        h = jnp.where((lane[:1] & 63) < R, h, 0.0)

        def gate(c0, cn):
            z = _rnd(jnp.sum(w2d[pl.ds(c0, cn), :] * h, axis=1, keepdims=True))
            return jnp.broadcast_to(_rnd(jax.nn.sigmoid(z)), (cn, 128))

        def apply(hh, c0, g):
            g = jnp.concatenate([g, g[:, :W - 128]], axis=1)
            for si in range(S):
                v = xbuf[si, hh, pl.ds(c0, CB), :].astype(F32)
                xbuf[si, hh, pl.ds(c0, CB), :] = (v * g).astype(xbuf.dtype)

        g0 = gate(0, CB)
        apply(0, 0, g0)
        gate_ref[pl.ds(0, CB), :] = g0
        wr(0, 0, CB).start()

        def row(hh, carry):
            for a in range(0, C, OUT_C):
                lo = max(a, CB)

                @pl.when(hh == 0)
                def _():
                    n = a + OUT_C - lo
                    gate_ref[pl.ds(lo, n), :] = gate(lo, n)

                if a == 0:
                    @pl.when(hh > 0)
                    def _():
                        apply(hh, 0, gate_ref[pl.ds(0, CB), :])

                for r in range(lo, a + OUT_C, CB):
                    apply(hh, r, gate_ref[pl.ds(r, CB), :])

                if a == 0:
                    @pl.when(hh == 0)
                    def _():
                        wr(0, CB, OUT_C - CB).start()

                    @pl.when(hh > 0)
                    def _():
                        wr(hh, 0, OUT_C).start()
                else:
                    wr(hh, a, OUT_C).start()
            return carry

        lax.fori_loop(0, HG, row, 0)
        pltpu.make_async_copy(xbuf, o_hbm, wsem).wait()

    xt = jnp.transpose(x, (0, 1, 3, 2)).reshape(S, HG, C, W)
    out = pl.pallas_call(
        kernel,
        out_shape=jax.ShapeDtypeStruct((S, HG, C, W), x.dtype),
        in_specs=[pl.BlockSpec(memory_space=pltpu.HBM)] * 3,
        out_specs=pl.BlockSpec(memory_space=pltpu.HBM),
        scratch_shapes=[
            pltpu.VMEM((S, HG, C, W), x.dtype),
            pltpu.VMEM((R, C), w1.dtype),
            pltpu.VMEM((R, C), w2.dtype),
            pltpu.VMEM((C, 128), F32),
            pltpu.VMEM((C, 128), F32),
            pltpu.VMEM((C, 128), F32),
            pltpu.SemaphoreType.DMA((len(reads),)),
            pltpu.SemaphoreType.DMA(()),
            pltpu.SemaphoreType.DMA((2,)),
        ],
        compiler_params=pltpu.CompilerParams(vmem_limit_bytes=64 * 1024 * 1024),
    )(xt, w1.T, w2)
    return jnp.transpose(out.reshape(B, H, C, W), (0, 1, 3, 2))
```
